```python
import os as _os
_os.environ.setdefault('JAX_PLATFORMS', 'cpu')
import jax
import jax.numpy as jnp

def _softmax(x, axis=-1):
    return jax.nn.softmax(x, axis=axis)

def _gelu(x):
    return jax.nn.gelu(x, approximate=True)

def _silu(x):
    return jax.nn.silu(x)

def _sigmoid(x):
    return jax.nn.sigmoid(x)

def _layernorm(x, axis=-1, eps=1e-05):
    m = jnp.mean(x, axis=axis, keepdims=True)
    v = jnp.var(x, axis=axis, keepdims=True)
    return (x - m) / jnp.sqrt(v + eps)

def _scatter_add(tgt, idx, src, axis=0):
    return tgt.at[idx].add(src)

def _segment_sum(src, seg, n):
    return jax.ops.segment_sum(src, seg, n)

class _Rng:

    def __init__(self, key):
        self._k = key

    def _next(self):
        self._k, sub = jax.random.split(self._k)
        return sub

    def normal(self, shape):
        return jax.random.normal(self._next(), shape, dtype=jnp.bfloat16)

    def randint(self, lo, hi, shape):
        return jax.random.randint(self._next(), shape, lo, hi, dtype=jnp.int32)

    def uniform(self, shape, lo=0.0, hi=1.0):
        return jax.random.uniform(self._next(), shape, jnp.bfloat16, lo, hi)

    def permutation(self, n):
        return jax.random.permutation(self._next(), n)
kernel_name = 'adaLN_cond__linear_attn_block__swiglu_ffn__prompt'

def setup_inputs():
    _rng = _Rng(jax.random.key(int.from_bytes(__import__("os").urandom(4), "little")))
    _w = lambda a: (lambda t: t.astype(jnp.bfloat16) if jnp.issubdtype(t.dtype, jnp.floating) else t)(jnp.asarray(a))

    def _A_setup():
        B, S, D = (1, 2048, 640)
        return {'x': _w((lambda *s: _rng.normal(s) * 0.05)(B, S, D)), 'wqkv': _w((lambda *s: _rng.normal(s) * 0.8)(D, 3 * D)), 'wo': _w((lambda *s: _rng.normal(s) * 0.05)(D, D))}
    _A_in = _A_setup()

    def _B_setup():
        B, S, D, F = (1, 2048, 640, 1728)
        return {'x': _w((lambda *s: _rng.normal(s) * 0.05)(B, S, D)), 'w_gate': _w((lambda *s: _rng.normal(s) * 0.05)(D, F)), 'w_up': _w((lambda *s: _rng.normal(s) * 0.05)(D, F)), 'w_down': _w((lambda *s: _rng.normal(s) * 0.05)(F, D))}
    _B_in = _B_setup()
    return {'A_x': _A_in['x'], 'A_wqkv': _A_in['wqkv'], 'A_wo': _A_in['wo'], 'B_x': _B_in['x'], 'B_w_gate': _B_in['w_gate'], 'B_w_up': _B_in['w_up'], 'B_w_down': _B_in['w_down'], 'c': _w((lambda *s: _rng.normal(s) * 0.05)(1, 640) * 8.0), 'w_mod': _w((lambda *s: _rng.normal(s) * 0.05)(640, 6 * 640) * 640 ** (-0.5) * 8.0)}

def reference(A_x, A_wqkv, A_wo, B_x, B_w_gate, B_w_up, B_w_down, c, w_mod):

    def _A_ref(x, wqkv, wo):
        B, S, D = x.shape
        H = 32
        Dh = D // H
        qkv = (lambda x, *d: x.transpose(*d))((x @ wqkv).reshape(B, S, 3, H, Dh), 2, 0, 3, 1, 4)
        q, k, v = (qkv[0], qkv[1], qkv[2])
        phi = lambda t: jnp.where(t > 0, t + 1, jnp.exp(t)) + 1e-06
        pq, pk = (phi(q), phi(k))
        kv = jnp.einsum('bhsd,bhse->bhde', pk, v)
        z = jnp.einsum('bhsd->bhd', pk)
        num = jnp.einsum('bhqd,bhde->bhqe', pq, kv)
        den = jnp.einsum('bhqd,bhd->bhq', pq, z)[..., None] + 1e-06
        o = num / den
        return (lambda x, *d: x.transpose(*d))(o, 0, 2, 1, 3).reshape(B, S, D) @ wo

    def _B_ref(x, w_gate, w_up, w_down):
        g = _silu(x @ w_gate)
        u = x @ w_up
        return g * u @ w_down
    x = A_x
    mod = (_silu(c) @ w_mod).reshape(c.shape[0], 6, 1, -1)
    sa, ca, ga, sb, cb, gb = (mod[:, 0].copy(), mod[:, 1].copy(), mod[:, 2].copy(), mod[:, 3].copy(), mod[:, 4].copy(), mod[:, 5].copy())
    h = _layernorm(x, axis=-1) * (1 + ca) + sa
    x = x + ga * _A_ref(h, A_wqkv, A_wo)
    h = _layernorm(x, axis=-1) * (1 + cb) + sb
    x = x + gb * _B_ref(h, B_w_gate, B_w_up, B_w_down)
    return x
```

```python
import jax, jax.numpy as jnp
from jax import lax
import jax.experimental.pallas as pl
import jax.experimental.pallas.tpu as pltpu

CFG = dict(TB=512, FC=1728)
bf16, f32 = jnp.bfloat16, jnp.float32
S, D, F, H, DH = 2048, 640, 1728, 32, 20


def dot(a, b): return jnp.dot(a, b, preferred_element_type=f32)
def dot_nt(a, b): return lax.dot_general(a, b, (((1,), (1,)), ((), ())), preferred_element_type=f32)
def phi(t): return jnp.where(t > 0, t + 1.0, jnp.exp(t)) + 1e-6
def lanes(col, n): return jnp.concatenate([col] * (n // 128), axis=1)


def layernorm_t(x):
    m = jnp.sum(x, axis=0, keepdims=True) * (1.0 / D)
    xc = x - m
    v = jnp.sum(xc * xc, axis=0, keepdims=True) * (1.0 / D)
    return xc * lax.rsqrt(v + 1e-5)


def kern(x_hbm, wqkv_hbm, wo_hbm, wg_hbm, wu_hbm, wd_hbm, c_ref, wmod_hbm, o_hbm,
         x_s, wqkv_s, wo_s, wg_s, wu_s, wd_s, wmod_s, o_s,
         modc, wkT, wqT, wdT, tmp, xT_s, pq_s, g_s, z_s, zp_s, wpT, y_s, sem, osem):
    TB, FC = CFG['TB'], CFG['FC']
    NB = S // TB
    cp = pltpu.make_async_copy
    d_x = [cp(x_hbm.at[pl.ds(i * TB, TB)], x_s.at[pl.ds(i * TB, TB)], sem.at[i]) for i in range(NB)]
    d_m0 = cp(wmod_hbm.at[:, pl.ds(0, 2 * D)], wmod_s.at[:, pl.ds(0, 2 * D)], sem.at[NB])
    d_wk = cp(wqkv_hbm.at[:, pl.ds(D, D)], wqkv_s.at[:, pl.ds(D, D)], sem.at[NB + 1])
    d_wq = cp(wqkv_hbm.at[:, pl.ds(0, D)], wqkv_s.at[:, pl.ds(0, D)], sem.at[NB + 2])
    d_wv = cp(wqkv_hbm.at[:, pl.ds(2 * D, D)], wqkv_s.at[:, pl.ds(2 * D, D)], sem.at[NB + 3])
    d_wo = cp(wo_hbm, wo_s, sem.at[NB + 4])
    d_m1 = cp(wmod_hbm.at[:, pl.ds(2 * D, 4 * D)], wmod_s.at[:, pl.ds(2 * D, 4 * D)], sem.at[NB + 5])
    d_wg = cp(wg_hbm, wg_s, sem.at[NB + 6])
    d_wu = cp(wu_hbm, wu_s, sem.at[NB + 7])
    d_wd = cp(wd_hbm, wd_s, sem.at[NB + 8])
    for d in [d_m0, d_x[0], d_wk, d_wq] + d_x[1:] + [d_wv, d_wo, d_m1, d_wg, d_wu, d_wd]:
        d.start()

    cf = c_ref[...].astype(f32)
    sc = jnp.broadcast_to(cf * jax.nn.sigmoid(cf), (16, D)).astype(bf16)

    def mod_cols(j0, j1):
        m = dot(sc, wmod_s[:, j0 * D:j1 * D])
        for j in range(j0, j1):
            for t in range(D // 128):
                o = (j - j0) * D + t * 128
                r = m[0:1, o:o + 128]
                if j in (1, 4):
                    r = r + 1.0
                modc[j, t * 128:(t + 1) * 128, :] = jnp.broadcast_to(r, (128, 128)).T
        return m

    d_m0.wait()
    mod_cols(0, 2)
    d_wk.wait()
    wkT[...] = wqkv_s[:, D:2 * D].T
    d_wq.wait()
    for t in range(5):
        tmp[t] = wqkv_s[t * 128:(t + 1) * 128, 0:D].astype(f32).T
    for d in range(DH):
        for t in range(5):
            wqT[d * H:(d + 1) * H, t * 128:(t + 1) * 128] = tmp[t, pl.ds(d, H, stride=DH), :].astype(bf16)
    g_s[...] = jnp.zeros(g_s.shape, f32)
    z_s[...] = jnp.zeros(z_s.shape, f32)

    def p1(i, _):
        for j in range(NB):
            @pl.when(i == j)
            def _():
                d_x[j].wait()
        xT = x_s[pl.ds(pl.multiple_of(i * TB, TB), TB), :].T
        xT_s[i] = xT
        h = (layernorm_t(xT.astype(f32)) * lanes(modc[1], TB) + lanes(modc[0], TB)).astype(bf16)
        pk = phi(dot(wkT[...], h))
        zz = pk[:, 0:128]
        for t in range(1, TB // 128):
            zz = zz + pk[:, t * 128:(t + 1) * 128]
        z_s[...] += zz
        pq_s[i] = phi(dot(wqT[...], h))
        g_s[...] += dot_nt(pk.astype(bf16), h)
    lax.fori_loop(0, NB, p1, None)

    d_wv.wait(); d_wo.wait(); d_m1.wait()
    m1 = mod_cols(2, 6)
    ga = m1[0:1, 0:D]
    kv = dot(g_s[...].astype(bf16), wqkv_s[:, 2 * D:3 * D])
    ri = lax.broadcasted_iota(jnp.int32, (D, D), 0)
    ci = lax.broadcasted_iota(jnp.int32, (D, D), 1)
    hd = lambda a: (a * 3277) >> 16
    kv = jnp.where(hd(ri) == hd(ci), kv, 0.0).astype(bf16)
    wp = dot(kv, wo_s[...]) * ga
    for t in range(5):
        tmp[t] = wp[:, t * 128:(t + 1) * 128]
    for t in range(5):
        wt = jnp.concatenate([tmp[t, pl.ds(d, H, stride=DH), :] for d in range(DH)], axis=0)
        wpT[t * 128:(t + 1) * 128, :] = wt.T.astype(bf16)
    z_s[...] = jnp.broadcast_to(jnp.sum(z_s[...], axis=1, keepdims=True), z_s.shape)
    for d in range(DH):
        zp_s[d * H:(d + 1) * H, :] = z_s[pl.ds(d, H, stride=DH), :]
    d_wd.wait()
    wdT[...] = wd_s[...].T
    d_wg.wait(); d_wu.wait()

    def out_copy(i):
        r = pl.ds(pl.multiple_of(i * TB, TB), TB)
        return cp(o_s.at[r], o_hbm.at[r], osem.at[i])

    def p2(i, _):
        pq = pq_s[i]
        zp = lanes(zp_s[...], TB)
        den = pq[0:H] * zp[0:H]
        for d in range(1, DH):
            den = den + pq[d * H:(d + 1) * H] * zp[d * H:(d + 1) * H]
        rden = 1.0 / (den + 1e-6)
        pqn = (pq * jnp.concatenate([rden] * DH, axis=0)).astype(bf16)
        x1 = xT_s[i].astype(f32) + dot(wpT[...], pqn)
        h = (layernorm_t(x1) * lanes(modc[4], TB) + lanes(modc[3], TB)).astype(bf16)
        for f0 in range(0, F, FC):
            g = dot(wg_s[f0:f0 + FC, :], h)
            u = dot(wu_s[f0:f0 + FC, :], h)
            hg = 0.5 * g
            y_s[f0:f0 + FC, :] = ((hg + hg * jnp.tanh(hg)) * u).astype(bf16)
        o = x1 + lanes(modc[5], TB) * dot(wdT[...], y_s[...])
        o_s[pl.ds(pl.multiple_of(i * TB, TB), TB), :] = o.astype(bf16).T
        out_copy(i).start()
    lax.fori_loop(0, NB, p2, None)
    for i in range(NB):
        out_copy(i).wait()


@jax.jit
def pallas_adaLN_cond__linear_attn_block__swiglu_ffn__prompt_kernel(A_x, A_wqkv, A_wo, B_x, B_w_gate, B_w_up, B_w_down, c, w_mod):
    TB = CFG['TB']; NB = S // TB
    hbm = pl.BlockSpec(memory_space=pl.ANY)
    V = pltpu.VMEM
    out = pl.pallas_call(
        kern, out_shape=jax.ShapeDtypeStruct((S, D), bf16),
        in_specs=[hbm] * 6 + [pl.BlockSpec(memory_space=pltpu.VMEM), hbm], out_specs=hbm,
        scratch_shapes=[V((S, D), bf16), V((D, 3 * D), bf16), V((D, D), bf16), V((F, D), bf16), V((F, D), bf16),
                        V((F, D), bf16), V((D, 6 * D), bf16), V((S, D), bf16),
                        V((6, D, 128), f32), V((D, D), bf16), V((D, D), bf16), V((D, F), bf16), V((5, D, 128), f32),
                        V((NB, D, TB), bf16), V((NB, D, TB), f32), V((D, D), f32), V((D, 128), f32), V((D, 128), f32),
                        V((D, D), bf16), V((F, TB), bf16),
                        pltpu.SemaphoreType.DMA((NB + 9,)), pltpu.SemaphoreType.DMA((NB,))],
        compiler_params=pltpu.CompilerParams(vmem_limit_bytes=110 * 2**20),
    )(A_x.reshape(S, D), A_wqkv, A_wo, B_w_gate.T, B_w_up.T, B_w_down, c, w_mod)
    return out.reshape(1, S, D)
```

```python
import jax
import jax.numpy as jnp
from jax import lax
import jax.experimental.pallas as pl
import jax.experimental.pallas.tpu as pltpu

bf16, f32, u32 = jnp.bfloat16, jnp.float32, jnp.uint32
S, D, F, DH = 2048, 640, 1728, 20
T = 128
TB = 4 * T
NB = S // TB
MQ = D // 4
FH, FQ = F // 2, F // 4
KD = 384
KR = (F - 4 * KD) // 2
ALL = slice(None)
ROWS_UP, ROWS_PROJ, ROWS_GRAM, ROWS_DOWN, ROWS_LAST = 48, (48, 48, 64), (80, 80), (96, 64), (64, 64, 32)
SPLIT = 384

SA = [(((1, 0), 1), ((0, 0), -1)), (((1, 0), 1), ((1, 1), 1)), (((1, 1), 1),), (((0, 0), 1), ((1, 1), 1)),
      (((0, 0), 1),), (((0, 0), 1), ((0, 1), 1)), (((0, 1), 1), ((1, 1), -1))]
SB = [(((0, 0), 1), ((0, 1), 1)), (((0, 0), 1),), (((1, 0), 1), ((0, 0), -1)), (((0, 0), 1), ((1, 1), 1)),
      (((0, 1), 1), ((1, 1), -1)), (((1, 1), 1),), (((1, 0), 1), ((1, 1), 1))]
SC = [(((1, 1), 1),), (((1, 0), 1), ((1, 1), -1)), (((0, 0), 1), ((1, 0), 1)), (((0, 0), 1), ((1, 1), 1)),
      (((0, 1), 1), ((1, 1), 1)), (((0, 0), -1), ((0, 1), 1)), (((0, 0), 1),)]
TA = [(((1, 0), 1), ((0, 0), -1)), (((1, 0), 1), ((1, 1), -1)), (((1, 1), 1),), (((0, 0), 1), ((1, 1), -1)),
      (((0, 0), 1),), (((0, 0), 1), ((0, 1), -1)), (((0, 1), 1), ((1, 1), -1))]
TP = (2, 1, 0, 3, 6, 5, 4)
TC = [(((1, 1), 1),), (((1, 0), 1), ((1, 1), 1)), (((0, 0), 1), ((1, 0), 1)), (((0, 0), 1), ((1, 1), -1)),
      (((0, 1), 1), ((1, 1), 1)), (((0, 0), -1), ((0, 1), -1)), (((0, 0), 1),)]
PLAIN = {(0, 0): 4 * 7 + 4, (1, 1): 4 * 7 + 2, (2, 2): 2 * 7 + 4, (3, 3): 2 * 7 + 2}
SPAN = ((0, 144), (112, 272), (240, 400), (368, 528), (496, 640))

BIG, SQUARE = (4, D, T), (5, D, T)
BUFFERS = dict(
    modr=(1, (6, 5, 8, T), f32), modc=(1, (6, D, T), f32), sc=(1, (D, T), f32),
    tw=(3, SQUARE, f32), wp=(1, SQUARE, f32), kv=(1, (5, MQ, T), bf16), g=(1, SQUARE, f32),
    x=(NB, BIG, f32), stats=(NB, (4, 2, 8, T), f32), h=(1, BIG, f32), p=(2, BIG, f32), y=(3, (2, 4, FH, T), f32),
    z=(2, (D, T), f32), zp=(1, (D, T), f32), inv=(2, (4, 4, 8, T), f32),
    ak=(1, (53, MQ, T), bf16), aq=(1, (53, MQ, T), bf16), ao=(1, (53, MQ, T), bf16), ap=(2, (65, MQ, T), bf16),
    ag=(2, (49, FQ, T), bf16), ad=(1, (49, 3, MQ, T), bf16), ad2=(1, (7, 2 * MQ, T), bf16),
    hb=(NB, (53, T, T), bf16), qb=(NB, (53, T, T), bf16), yb=(3, (49, KD, T), bf16), yb2=(3, (7, 2, T, T), bf16))


def dot(a, b): return jnp.dot(a, b, preferred_element_type=f32)
def dot_nt(a, b): return lax.dot_general(a, b, (((1,), (1,)), ((), ())), preferred_element_type=f32)
def phi(t): return jnp.where(t > 0, t + 1.0, jnp.exp(t)) + 1e-6
def rng(r0, n): return slice(r0, r0 + n)
def tile(t): return rng(t * T, T)
def spans(sizes): return [(sum(sizes[:n]), size) for n, size in enumerate(sizes)]
def tree(xs): return xs[0] if len(xs) == 1 else tree(xs[:len(xs) // 2]) + tree(xs[len(xs) // 2:])


def ld(ref, *idx):
    *lead, (r0, n) = idx
    return pltpu.bitcast(ref.bitcast(u32)[(*lead, rng(r0 // 2, n // 2), ALL)], bf16)


def level(get, terms, h):
    out = {}
    for r in range(h):
        for c in range(h):
            (i, j), _ = terms[0]
            v = get(i * h + r, j * h + c)
            for (i, j), s in terms[1:]:
                w = get(i * h + r, j * h + c)
                v = v + w if s > 0 else v - w
            out[r, c] = v
    return out


def sums(get, put, table, levels, nrows):
    for p, terms in enumerate(table):
        for r0 in range(0, nrows, 16):
            sub = level(lambda i, j: get(i, j, r0), terms, levels)
            if levels == 1:
                put(p, r0, sub[0, 0].astype(bf16))
            else:
                for q, inner in enumerate(table):
                    put(7 * p + q, r0, level(lambda i, j: sub[i, j], inner, 1)[0, 0].astype(bf16))
            yield


def n_sums(nrows): return 7 * nrows // 16


def products(mul, levels, table, done, init=None, base=0):
    if levels == 0:
        v = mul(base)
        yield
        yield from done((0, 0), v) or ()
        return
    last = {ij: p for p, terms in enumerate(table) for ij, _ in terms}
    acc = {}
    for p, terms in enumerate(table):
        def take(rc, v):
            for (i, j), s in terms:
                key = (i * levels + rc[0], j * levels + rc[1])
                if key not in acc and init is not None:
                    acc[key] = init(*key)
                    yield
                if key not in acc:
                    assert s > 0
                    acc[key] = v
                else:
                    acc[key] = acc[key] + v if s > 0 else acc[key] - v
                if last[i, j] == p:
                    yield from done(key, acc.pop(key)) or ()
        yield from products(mul, levels - 1, table, take, None, base * 7 + p)


def chain(*jobs):
    return (step for gen, _ in jobs for step in gen), sum(n for _, n in jobs)


def run(main, *side):
    pos = [0] * len(side)
    for step, _ in enumerate(main[0], 1):
        for k, (gen, n) in enumerate(side):
            while pos[k] * main[1] < step * n and pos[k] < n:
                next(gen, None)
                pos[k] += 1
    for gen, _ in side:
        for _ in gen:
            pass


class Copy:
    def __init__(self, hbm, vmem, tiles, sem, rows=ALL, out=False):
        pairs = [(hbm.at[rows, tile(t)], vmem.at[t, rows]) for t in tiles]
        self.parts = [pltpu.make_async_copy(*(p[::-1] if out else p), sem) for p in pairs]

    def start(self):
        for p in self.parts:
            p.start()

    def wait(self):
        for p in self.parts:
            p.wait()


def kernel(x_hbm, wqkv_hbm, wo_hbm, wg_hbm, wu_hbm, wd_hbm, c_hbm, wmod_hbm, o_hbm,
           x_s, wqkv_s, wo_s, wg_s, wu_s, wd_s, wmod_s, o_s, c_s, bufs, sem, osem):
    def buf(name, i=0): return bufs[name][i % len(bufs[name])]

    def silu_c():
        c = c_s[...].astype(f32)
        return c * jax.nn.sigmoid(c)

    def mod_rows_mxu(j):
        sc = jnp.broadcast_to(silu_c(), (16, D)).astype(bf16)
        for t in range(5):
            buf('modr')[j, t] = dot(sc, ld(wmod_s, 5 * j + t, (0, D)))[0:8]
            yield

    def mod_rows_vpu(*js):
        for j in js:
            for t in range(5):
                acc = []
                for r0 in range(0, D, 64):
                    w = ld(wmod_s, 5 * j + t, (r0, 64)).astype(f32) * buf('sc')[rng(r0, 64), :]
                    acc.append(tree([w[r:r + 8] for r in range(0, 64, 8)]))
                buf('modr')[j, t] = jnp.broadcast_to(jnp.sum(tree(acc), axis=0, keepdims=True), (8, T))
                yield

    def mod_cols(*js):
        for j in js:
            for t in range(5):
                r = buf('modr')[j, t]
                r = (r, r + 1.0, None, r * 0.5, (r + 1.0) * 0.5, r * 2.0)[j]
                buf('modc')[j, tile(t), :] = jnp.concatenate([r] * (T // 8), axis=0).T
                yield

    def sums_a(dst, get):
        for i in range(4):
            dst[49 + i] = get(4, i * MQ, MQ).astype(bf16)
            yield

        def put(p, r0, v): dst[p, rng(r0, 16), :] = v
        yield from sums(lambda i, k, r0: get(k, i * MQ + r0, 16), put, SA, 2, MQ)

    def sums_b(dst, get):
        for j in range(4):
            dst[49 + j] = get(j, 4 * T, T).astype(bf16)
            yield

        def put(p, r0, v): dst[p, rng(r0, 16), :] = v
        yield from sums(lambda k, j, r0: get(j, k * T + r0, 16), put, SB, 2, T)
    n_a, n_b = 4 + n_sums(MQ), 4 + n_sums(T)

    def by_dim(ref, lead, r0, n):
        return jnp.concatenate([ref[(*lead, pl.ds(r // MQ * MQ + r % MQ // 8, 8, stride=DH), ALL)]
                                for r in range(r0, r0 + n, 8)], axis=0)

    def flip_w(slot, m0):
        for m in range(5):
            for k in range(5):
                buf('tw', slot)[k, tile(m), :] = ld(wqkv_s, m0 + m, (k * T, T)).astype(f32).T
                yield

    class Stats:
        def __init__(self, i):
            self.dst, self.acc = buf('stats', i), {}

        def add(self, j, v):
            shift, s1, s2, n = self.acc.get(j, (jnp.broadcast_to(v[0:1], (8, T)), None, None, 0))
            d = [v[r:r + 8] - shift for r in range(0, v.shape[0], 8)]
            t1, t2 = tree(d), tree([e * e for e in d])
            s1, s2 = (t1, t2) if s1 is None else (s1 + t1, s2 + t2)
            self.acc[j] = shift, s1, s2, n + v.shape[0]
            if n + v.shape[0] == D:
                m = jnp.sum(s1, axis=0, keepdims=True) * (1.0 / D)
                var = jnp.maximum(jnp.sum(s2, axis=0, keepdims=True) * (1.0 / D) - m * m, 0.0)
                self.dst[j, 0] = jnp.broadcast_to(lax.rsqrt(var + 1e-5), (8, T))
                self.dst[j, 1] = shift + m

    def flip_x(i):
        st = Stats(i)
        for j in range(4):
            for k in range(5):
                v = ld(x_s, k, (i * TB + j * T, T)).astype(f32).T
                buf('x', i)[j, tile(k), :] = v
                st.add(j, v)
                yield

    def norm(i, scale, shift):
        src, st, mod = buf('x', i), buf('stats', i), buf('modc')
        for j in range(4):
            rs, m = (jnp.concatenate([st[j, a]] * 4, axis=0) for a in range(2))
            for r0 in range(0, D, 32):
                r = rng(r0, 32)
                buf('h')[j, r, :] = (src[j, r, :] - m) * rs * mod[scale, r, :] + mod[shift, r, :]
                yield

    def project(a, b, done):
        for r0, n in spans(ROWS_PROJ):
            yield from products(lambda p: dot(ld(a, p, (r0, n)), ld(b, p, (0, T))), 2, SC,
                                lambda key, v: done(key[0], key[1], key[0] * MQ + r0, v),
                                lambda r, c: dot(ld(a, 49 + r, (r0, n)), ld(b, 49 + c, (0, T))))

    def k_proj(i):
        part = {}

        def done(r, j, r0, v):
            p, rows = phi(v), rng(r0, v.shape[0])
            buf('p', i)[j, rows, :] = p
            n, z = part.pop(r0, (0, buf('z', i - 1)[rows, :] if i else None))
            z = p if z is None else z + p
            if n == 3:
                buf('z', i)[rows, :] = z
            else:
                part[r0] = (n + 1, z)
        yield from project(buf('ak'), buf('hb', i), done)

    def sums_k(i):
        src, dst = buf('p', i), buf('ap', i)
        for r in range(4):
            for r0 in range(0, MQ, 32):
                for j in range(4):
                    if (r, j) not in PLAIN:
                        dst[49 + 4 * r + j, rng(r0, 32), :] = src[j, rng(r * MQ + r0, 32), :].astype(bf16)
                yield

        def put(p, r0, v): dst[p, rng(r0, 16), :] = v
        yield from sums(lambda r, j, r0: src[j, rng(r * MQ + r0, 16), :], put, TA, 2, MQ)

    def gram(i):
        a, b, g = buf('ap', i), buf('hb', i), buf('g')
        for r0, n in spans(ROWS_GRAM):
            for r in range(4):
                rows = rng(r * MQ + r0, n)
                acc = g[4, rows, :] if i else None
                for k in range(4):
                    v = dot_nt(ld(a, PLAIN.get((r, k), 49 + 4 * r + k), (r0, n)), ld(b, 49 + k, (0, T)))
                    acc = v if acc is None else acc + v
                    yield
                g[4, rows, :] = acc

            def done(key, v):
                rows = rng(key[0] * MQ + r0, n)
                g[key[1], rows, :] = v + g[key[1], rows, :] if i else v
            yield from products(lambda p: dot_nt(ld(a, p, (r0, n)), ld(b, TP[p // 7] * 7 + TP[p % 7], (0, T))),
                                2, TC, done)

    def prep_z():
        buf('z', NB)[...] = jnp.broadcast_to(jnp.sum(buf('z', NB - 1)[...], axis=1, keepdims=True), (D, T))
        yield
        buf('zp')[...] = by_dim(buf('z', NB), (), 0, D)
        yield

    def q_proj(i):
        den = {}

        def done(r, j, r0, v):
            p, n = phi(v), v.shape[0]
            buf('p', i)[j, rng(r0, n), :] = p
            w = p * buf('zp')[rng(r0, n), :]
            w = tree([w[d:d + 8] for d in range(0, n, 8)])
            den[r, j] = w + den[r, j] if (r, j) in den else w
            if r0 + n == (r + 1) * MQ:
                buf('inv', i)[r, j] = 1.0 / (den[r, j] + 1e-6)
        yield from project(buf('aq'), buf('hb', i), done)

    def sums_q(i):
        def get(j, r0, n):
            inv = jnp.concatenate([buf('inv', i)[r // MQ, j] for r in range(r0, r0 + n, 8)], axis=0)
            return buf('p', i)[j, rng(r0, n), :] * inv
        yield from sums_b(buf('qb', i), get)

    def prep_kv():
        for t, (lo, hi) in enumerate(SPAN):
            g = jnp.concatenate([buf('g')[k, lo:hi, :] for k in range(5)], axis=1).astype(bf16)
            kv = dot(g, ld(wqkv_s, 10 + t, (0, D)))
            row = lax.broadcasted_iota(jnp.int32, kv.shape, 0) + lo
            col = lax.broadcasted_iota(jnp.int32, kv.shape, 1) + t * T
            same_head = (row * 3277) >> 16 == (col * 3277) >> 16
            buf('kv')[t, 0:hi - lo, :] = jnp.where(same_head, kv, 0.0).astype(bf16)
            yield
        for m in range(5):
            keep = None
            for t, (lo, hi) in enumerate(SPAN):
                old = SPAN[t - 1][1] - lo if t else 0
                end = SPAN[t + 1][0] if t < 4 else hi
                w = dot(ld(buf('kv'), t, (0, hi - lo)), ld(wo_s, m, (t * T, T))) * buf('modr')[2, m, 0:1, :]
                if old:
                    buf('wp')[m, lo:lo + old, :] = w[:old] + keep
                buf('wp')[m, lo + old:end, :] = w[old:end - lo]
                keep = w[end - lo:] if t < 4 else None
                yield

    def flip_o():
        for k in range(5):
            for m in range(5):
                buf('tw', 2)[k, tile(m), :] = by_dim(buf('wp'), (m,), k * T, T).T
                yield

    def attn(i):
        x, st = buf('x', i), Stats(i)

        def done(r, j, r0, v):
            rows = rng(r0, v.shape[0])
            v = x[j, rows, :] + v
            x[j, rows, :] = v
            st.add(j, v)
        yield from project(buf('ao'), buf('qb', i), done)

    R, w_up = ROWS_UP, (wg_s, wu_s)

    def sums_up(lo, hi):
        for unit in range(lo // R, hi // R):
            w, c0 = unit % 2, unit // 2 * R

            def put(p, r0, v): buf('ag', w)[p, rng(c0 + r0, 16), :] = v
            yield from sums(lambda i, k, r0: ld(w_up[w], k, (i * FQ + c0 + r0, 16)).astype(f32), put, SA, 2, R)

    def gate_up(i, lo, hi):
        b = buf('hb', i)
        for r0 in range(lo // 2, hi // 2, R):
            act = {}

            def gate(key, g): act[key] = g + g * jnp.tanh(g)

            def up(key, u):
                r, j = key
                buf('y', i)[r // 2, j, rng(r % 2 * FQ + r0, R), :] = act.pop(key) * u
            for w, done in enumerate((gate, up)):
                yield from products(lambda p: dot(ld(buf('ag', w), p, (r0, R)), ld(b, p, (0, T))), 2, SC, done,
                                    lambda r, c: dot(ld(w_up[w], 4, (r * FQ + r0, R)), ld(b, 49 + c, (0, T))))

    def sums_y(i):
        y = buf('y', i)
        for t in range(2):
            def put(p, r0, v): buf('yb2', i)[p, t, rng(r0, 16), :] = v
            yield from sums(lambda g, j, r0: y[g, 2 * j + t, rng(2 * KD + r0, 16), :], put, SB, 1, KR)
        for c0 in range(0, KD, 32):
            def put(p, r0, v): buf('yb', i)[p, rng(c0 + r0, 16), :] = v
            yield from sums(lambda q, j, r0: y[q // 2, j, rng(q % 2 * KD + c0 + r0, 16), :], put, SB, 2, 32)

    def out_rows(r, r0):
        return rng(r0 // 32 * T + r * 32 + r0 % 32, 16)

    def prep_down():
        for kt in range(3):
            for q in range(4):
                for m in range(5):
                    buf('tw', kt)[q, tile(m), :] = ld(wd_s, m, (q // 2 * FH + q % 2 * KD + kt * T, T)).astype(f32).T
                    yield
        for q in range(2):
            for m in range(5):
                w = ld(wd_s, m, (q * FH + 2 * KD, KR)).astype(f32)
                buf('wp')[q, tile(m), :] = jnp.concatenate([w, jnp.zeros((T - KR, T), f32)], axis=0).T
                yield
        for a in range(2):
            def put(p, r0, v): buf('ad2')[p, rng(a * MQ + r0, 16), :] = v
            yield from sums(lambda i, q, r0: buf('wp')[q, out_rows(2 * i + a, r0), :], put, SA, 1, MQ)
        for kt in range(3):
            def put(p, r0, v): buf('ad')[p, kt, rng(r0, 16), :] = v
            yield from sums(lambda i, q, r0: buf('tw', kt)[q, out_rows(i, r0), :], put, SA, 2, MQ)

    def chunks(i): return spans(ROWS_LAST if i == NB - 1 else ROWS_DOWN)
    d_out = [[Copy(o_hbm, o_s, range(r0 // 32, (r0 + n) // 32), osem.at[5 * i + r0 // 32], rng(i * TB, TB), out=True)
              for r0, n in chunks(i)] for i in range(NB)]

    def down(i):
        a, a2, b, b2 = buf('ad'), buf('ad2'), buf('yb', i), buf('yb2', i)
        for c, (r0, n) in enumerate(chunks(i)):
            rest, ready = {}, {}
            for u in range(2):
                for t in range(2):
                    def keep(key, v): rest[2 * key[0] + u, 2 * key[1] + t] = v
                    yield from products(lambda p: dot(ld(a2, p, (u * MQ + r0, n)), ld(b2, p, t, (0, T))), 1, SC, keep)

            def done(key, v):
                j = key[1]
                ready[key] = v
                if all((q, j) in ready for q in range(4)):
                    for r in range(0, n, 32):
                        k = (r0 + r) // 32
                        v = jnp.concatenate([ready[q, j][r:r + 32] for q in range(4)], axis=0)
                        v = buf('x', i)[j, tile(k), :] + buf('modc')[5, tile(k), :] * v
                        o_s[k, rng(i * TB + j * T, T), :] = v.astype(bf16).T
            yield from products(lambda p: dot(jnp.concatenate([ld(a, p, t, (r0, n)) for t in range(3)], axis=1),
                                              ld(b, p, (0, KD))), 2, SC, done, lambda r, j: rest.pop((r, j)))
            if i == NB - 1:
                d_out[i][c].start()

    def K(i): return k_proj(i), 65 * len(ROWS_PROJ)
    def Q(i): return q_proj(i), 65 * len(ROWS_PROJ)
    def A(i): return attn(i), 65 * len(ROWS_PROJ)
    def G(i): return gram(i), 65 * len(ROWS_GRAM)
    def U(i, lo=0, hi=FH): return gate_up(i, lo, hi), 65 * (hi - lo) // R
    def Dn(i): return down(i), 93 * len(chunks(i))
    def FX(i): return flip_x(i), 20
    def N1(i): return norm(i, 1, 0), 80
    def N2(i): return norm(i, 4, 3), 80
    def SH(i): return sums_b(buf('hb', i), lambda j, r0, n: buf('h')[j, rng(r0, n), :]), n_b
    def SK(i): return sums_k(i), 20 + n_sums(MQ)
    def SQ(i): return sums_q(i), n_b
    def SY(i): return sums_y(i), 2 * n_sums(KR) + n_sums(KD)
    def WU(lo, hi): return sums_up(lo, hi), n_sums(hi - lo)
    wk = chain((flip_w(0, 5), 25), (sums_a(buf('ak'), lambda k, r0, n: buf('tw', 0)[k, rng(r0, n), :]), n_a))
    wq = sums_a(buf('aq'), lambda k, r0, n: by_dim(buf('tw', 1), (k,), r0, n)), n_a
    wo = sums_a(buf('ao'), lambda k, r0, n: buf('tw', 2)[k, rng(r0, n), :]), n_a

    d_x = [Copy(x_hbm, x_s, range(5), sem.at[i], rng(i * TB, TB)) for i in range(NB)]
    d_sa, d_ca, d_mod, d_wq, d_wk, d_wv, d_wo, d_wg, d_wu, d_wd = (
        Copy(hbm, vmem, tiles, sem.at[NB + n]) for n, (hbm, vmem, tiles) in enumerate((
            (wmod_hbm, wmod_s, range(5)), (wmod_hbm, wmod_s, range(5, 10)), (wmod_hbm, wmod_s, range(10, 30)),
            (wqkv_hbm, wqkv_s, range(5)), (wqkv_hbm, wqkv_s, range(5, 10)), (wqkv_hbm, wqkv_s, range(10, 15)),
            (wo_hbm, wo_s, range(5)), (wg_hbm, wg_s, range(5)), (wu_hbm, wu_s, range(5)), (wd_hbm, wd_s, range(5)))))
    d_c = pltpu.make_async_copy(c_hbm, c_s, sem.at[NB + 10])

    first = [(d_sa, chain((mod_rows_mxu(0), 5), (mod_cols(0), 5))), (d_ca, chain((mod_rows_mxu(1), 5), (mod_cols(1), 5))),
             (d_x[0], chain(FX(0), N1(0), SH(0))), (d_wk, wk), (d_x[1], FX(1))]
    for d in [d_c, *[d for d, _ in first], d_x[2], d_x[3]]:
        d.start()
    for i in range(3):
        buf('yb2', i)[:, :, KR:, :] = jnp.zeros((7, 2, T - KR, T), bf16)
    d_c.wait()
    for t in range(5):
        buf('sc')[tile(t), :] = jnp.broadcast_to(silu_c()[:, tile(t)], (T, T)).T
    zero = jnp.max(pltpu.bitcast(c_s[:, 0:T].astype(f32), jnp.int32) & 0xFFFF)
    pl.when(zero == 1)(lambda: run(chain(*[G(i % NB) for i in range(4)])))
    for d, job in first:
        d.wait()
        run(job)

    def stage(main, *side, start=(), wait=()): return main, side, start, wait
    stages = [
        stage(K(0), chain(N1(1), SH(1)), start=[d_wq, d_mod]),
        stage(K(1), SK(0), FX(2), start=[d_wg, d_wu], wait=[d_x[2]]),
        stage(G(0), N1(2), SK(1), start=[d_wv, d_wo, d_wd]),
        stage(G(1), SH(2), FX(3), wait=[d_x[3]]),
        stage(K(2), chain(N1(3), SH(3))),
        stage(K(3), SK(2), (flip_w(1, 0), 25), wait=[d_wq]),
        stage(G(2), SK(3), (prep_z(), 2), wq),
        stage(chain(G(3), Q(0)), (mod_rows_vpu(2, 3, 4), 15), wait=[d_mod]),
        stage(Q(1), (prep_kv(), 30), SQ(0), *([WU(0, 48)] if R == 48 else []), wait=[d_wg, d_wu, d_wv, d_wo]),
        stage(Q(2), (flip_o(), 25), SQ(1)),
        stage(Q(3), wo, (mod_cols(3, 4), 10), WU(48 if R == 48 else 0, 96)),
        stage(chain(A(0), A(1)), SQ(2), SQ(3), WU(96, 288)),
        stage(A(2), chain(N2(0), SH(0)), WU(288, SPLIT)),
        stage(chain(A(3), U(0, 0, SPLIT)), WU(SPLIT, FH), chain(N2(1), SH(1))),
        stage(chain(U(0, SPLIT), U(1)), (prep_down(), 70 + 5 * n_sums(MQ)), chain(N2(2), SH(2), N2(3), SH(3)),
              chain((mod_rows_vpu(5), 5), (mod_cols(5), 5)), wait=[d_wd]),
        stage(U(2), SY(0), SY(1)),
        stage(chain(Dn(0), U(3)), SY(2)),
        stage(chain(Dn(1), Dn(2)), SY(3), start=d_out[0]),
        stage(Dn(3), start=d_out[1] + d_out[2]),
    ]
    for n, (main, side, start, wait) in enumerate(stages):
        for d in start:
            d.start()
        for d in wait:
            d.wait()
        pl.when(zero * (n + 2) == 0)(lambda: run(main, *side))
    for ds in d_out:
        for d in ds:
            d.wait()


@jax.jit
def pallas_adaLN_cond__linear_attn_block__swiglu_ffn__prompt_kernel(
    A_x: jax.Array, A_wqkv: jax.Array, A_wo: jax.Array, B_x: jax.Array, B_w_gate: jax.Array,
    B_w_up: jax.Array, B_w_down: jax.Array, c: jax.Array, w_mod: jax.Array,
):
    del B_x
    hbm = pl.BlockSpec(memory_space=pl.ANY)
    staged = ((S, D), (D, 3 * D), (D, D), (F, D), (F, D), (F, D), (D, 6 * D), (S, D))
    out = pl.pallas_call(
        kernel,
        out_shape=jax.ShapeDtypeStruct((S, D), bf16),
        in_specs=[hbm] * 8,
        out_specs=hbm,
        scratch_shapes=[pltpu.VMEM((n // T, m, T), bf16) for m, n in staged] + [
            pltpu.VMEM((1, D), bf16),
            {k: [pltpu.VMEM(shape, dt) for _ in range(n)] for k, (n, shape, dt) in BUFFERS.items()},
            pltpu.SemaphoreType.DMA((NB + 11,)), pltpu.SemaphoreType.DMA((5 * NB,))],
        compiler_params=pltpu.CompilerParams(
            vmem_limit_bytes=116 * 2**20, flags={'XLA_TPU_EVENLY_DISTRIBUTE_CRITICAL_NODES': True}),
    )(A_x.reshape(S, D), A_wqkv, A_wo, B_w_gate.T, B_w_up.T, B_w_down, c, w_mod)
    return out.reshape(1, S, D)
```
